```python
import os as _os
_os.environ.setdefault('JAX_PLATFORMS', 'cpu')
import jax
import jax.numpy as jnp

def _softmax(x, axis=-1):
    return jax.nn.softmax(x, axis=axis)

def _gelu(x):
    return jax.nn.gelu(x, approximate=True)

def _silu(x):
    return jax.nn.silu(x)

def _sigmoid(x):
    return jax.nn.sigmoid(x)

def _layernorm(x, axis=-1, eps=1e-05):
    m = jnp.mean(x, axis=axis, keepdims=True)
    v = jnp.var(x, axis=axis, keepdims=True)
    return (x - m) / jnp.sqrt(v + eps)

def _scatter_add(tgt, idx, src, axis=0):
    return tgt.at[idx].add(src)

def _segment_sum(src, seg, n):
    return jax.ops.segment_sum(src, seg, n)

class _Rng:

    def __init__(self, key):
        self._k = key

    def _next(self):
        self._k, sub = jax.random.split(self._k)
        return sub

    def normal(self, shape):
        return jax.random.normal(self._next(), shape, dtype=jnp.bfloat16)

    def randint(self, lo, hi, shape):
        return jax.random.randint(self._next(), shape, lo, hi, dtype=jnp.int32)

    def uniform(self, shape, lo=0.0, hi=1.0):
        return jax.random.uniform(self._next(), shape, jnp.bfloat16, lo, hi)

    def permutation(self, n):
        return jax.random.permutation(self._next(), n)
kernel_name = 'standalone__conformer_conv_module__speech'

def setup_inputs():
    _rng = _Rng(jax.random.key(int.from_bytes(__import__("os").urandom(4), "little")))
    _w = lambda a: (lambda t: t.astype(jnp.bfloat16) if jnp.issubdtype(t.dtype, jnp.floating) else t)(jnp.asarray(a))
    B, T, D, K = (2, 4000, 512, 15)
    return {'x': _w((lambda *s: _rng.normal(s) * 0.2)(B, T, D)), 'w_pw1': _w((lambda *s: _rng.normal(s) * 0.2)(D, 2 * D)), 'dw': _w((lambda *s: _rng.normal(s) * 0.05)(K, D)), 'w_pw2': _w((lambda *s: _rng.normal(s) * 0.05)(D, D))}

def reference(x, w_pw1, dw, w_pw2):
    B, T, D = x.shape
    K = dw.shape[0]
    h = x @ w_pw1
    a, b = (h[..., :D].copy(), h[..., D:].copy())
    h = a * _sigmoid(b)
    pad = K // 2
    hp = jnp.pad(h, ((0, 0), (pad, pad), (0, 0)))
    out = jnp.zeros_like(h)
    for i in range(K):
        out = out + hp[:, i:i + T, :] * dw[i][None, None, :]
    return _silu(out) @ w_pw2
```

```python
import jax
import jax.numpy as jnp
from jax import lax
import jax.experimental.pallas as pl
import jax.experimental.pallas.tpu as pltpu

LANES = 128
CHUNK = 80
CHUNKS = 10
TILE = CHUNK * CHUNKS
AHEAD = 16
HALO = 8
C_LAG = 8
OUT_GROUPS = (0, 5, 8, 9, 10)
HEAD_COLS = 2
HEAD_CHUNKS = (3, 4)


def _interleave(a_pieces, c_pieces, lag):
    prog = []
    todo = list(c_pieces)
    for n, (j, c) in enumerate(a_pieces):
        prog += [("A", j, c), ("B", j, c)]
        if n >= lag and todo:
            prog.append(("C",) + todo.pop(0))
    return prog + [("C",) + p for p in todo]


def _join(prog, sync, rest):
    return prog[:-1] + [sync, prog[-1]] + rest


@jax.jit
def pallas_standalone__conformer_conv_module__speech_kernel(
    x: jax.Array,
    w_pw1: jax.Array,
    dw: jax.Array,
    w_pw2: jax.Array,
):
    batch, seq, dim = x.shape
    taps = dw.shape[0]
    pad = taps // 2
    rows = batch * seq
    nc = dim // LANES
    tiles = rows // TILE
    tiles_per_seq = seq // TILE
    assert dim % LANES == 0 and nc > HEAD_COLS and pad <= HALO
    assert seq % TILE == 0 and tiles_per_seq > 1 and tiles % 2 == 0
    f32, bf16, u32 = jnp.float32, jnp.bfloat16, jnp.uint32
    pieces = [(j, c) for j in range(CHUNKS) for c in range(nc)]

    def kernel(x_hbm, w1_hbm, dw_hbm, w2_hbm, o_hbm,
               x_even, x_odd, w1_v, dw_v, w2_v, dw_f, o_v, h_v, carry_v,
               head_sem, x_sem, o_sem):
        def cols(c):
            return pl.ds(c * LANES, LANES)

        def aligned(r):
            return r if isinstance(r, int) else pl.multiple_of(r, AHEAD)

        def start(copies):
            for cp in copies:
                cp.start()

        def wait(copies):
            for cp in copies:
                cp.wait()

        def x_copies(src_row, n, buf, dst_row, sem):
            return [
                pltpu.make_async_copy(
                    x_hbm.at[pl.ds(aligned(src_row), n), cols(c)],
                    buf.at[c, pl.ds(dst_row, n)], sem)
                for c in range(nc)
            ]

        def start_x_tile(i, buf, sem, may_be_last=False):
            r = i * TILE + AHEAD
            if not may_be_last:
                start(x_copies(r, TILE, buf, AHEAD, sem))
                return
            start(x_copies(r, TILE - AHEAD, buf, AHEAD, sem))
            start(x_copies(jnp.minimum(r + TILE - AHEAD, rows - AHEAD), AHEAD, buf, TILE, sem))

        def wait_x_tile(buf, sem):
            filled = buf.at[:, pl.ds(AHEAD, TILE)]
            pltpu.make_async_copy(filled, filled, sem).wait()

        def packed(v):
            return pltpu.bitcast(v, bf16)

        w1_w, w2_w = w1_v.bitcast(u32), w2_v.bitcast(u32)

        def run(i, x_buf, prog, seq_end):
            head = isinstance(i, int)
            x_w = x_buf.bitcast(u32)
            act, lhs, done = {}, {}, [0] * CHUNKS

            def piece_a(j, c):
                lo = 0 if head and j == 0 else AHEAD + j * CHUNK
                hi = AHEAD + (j + 1) * CHUNK
                xt = jnp.concatenate(
                    [packed(x_w[k, lo // 2:hi // 2, :]) for k in range(nc)], axis=1)
                b = jnp.dot(xt, packed(w1_w[nc + c]), preferred_element_type=f32)
                a = jnp.dot(xt, packed(w1_w[c]), preferred_element_type=f32)
                h = a * jnp.tanh(b * 0.5) + a
                if j < CHUNKS - 1:
                    h_v[c, HALO + lo:HALO + hi, :] = h
                    return
                own = CHUNK - AHEAD
                nxt = h[own:own + HALO]
                h_v[c, HALO + lo:HALO + TILE, :] = h[:own]
                h_v[c, HALO + TILE:, :] = nxt if head else jnp.where(seq_end, 0.0, nxt)
                carry_v[c] = h[own:]

            def piece_b(j, c):
                y = None
                for k in range(taps):
                    r = HALO - pad + j * CHUNK + k
                    t = h_v[c, r:r + CHUNK, :] * dw_f[k:k + 1, cols(c)]
                    y = t if y is None else y + t
                act[j, c] = y * jnp.tanh(y) + y

            def piece_c(j, c):
                if j not in lhs:
                    lhs[j] = jnp.concatenate(
                        [act[j, k] for k in range(nc)], axis=1).astype(bf16)
                out = jnp.dot(lhs[j], packed(w2_w[c]), preferred_element_type=f32)
                o_v[c, pl.ds(aligned(i * TILE + j * CHUNK), CHUNK), :] = out.astype(bf16)
                done[j] += 1
                if done[j] == nc and j + 1 in OUT_GROUPS:
                    j0 = OUT_GROUPS[OUT_GROUPS.index(j + 1) - 1]
                    span = pl.ds(aligned(i * TILE + j0 * CHUNK), (j + 1 - j0) * CHUNK)
                    start([
                        pltpu.make_async_copy(o_v.at[k, span], o_hbm.at[span, cols(k)], o_sem)
                        for k in range(nc)
                    ])

            for op in prog:
                if callable(op):
                    op()
                else:
                    {"A": piece_a, "B": piece_b, "C": piece_c}[op[0]](op[1], op[2])

        j1, j2 = HEAD_CHUNKS
        edges = [0, AHEAD + j1 * CHUNK, AHEAD + j2 * CHUNK, AHEAD + TILE]
        x_head = [
            x_copies(edges[p], edges[p + 1] - edges[p], x_even, edges[p], head_sem.at[p])
            for p in range(3)
        ]

        def w1_copies(blocks, sem):
            return [
                pltpu.make_async_copy(w1_hbm.at[:, cols(q)], w1_v.at[q], sem)
                for c in blocks for q in (nc + c, c)
            ]

        phase = [
            x_head[0] + w1_copies(range(HEAD_COLS), head_sem.at[0]),
            w1_copies(range(HEAD_COLS, nc), head_sem.at[1]) + x_head[1],
            [
                pltpu.make_async_copy(w2_hbm.at[:, cols(c)], w2_v.at[c], head_sem.at[2])
                for c in range(nc)
            ] + x_head[2],
        ]
        dw_copy = pltpu.make_async_copy(dw_hbm, dw_v, head_sem.at[3])
        dw_copy.start()
        for copies in phase:
            start(copies)
        for c in range(nc):
            h_v[c, 0:HALO, :] = jnp.zeros((HALO, LANES), f32)
        dw_copy.wait()
        dw_f[...] = dw_v[...].astype(f32) * 0.25
        wait(phase[0])

        def sync2():
            wait(phase[1])

        def sync3():
            start_x_tile(1, x_odd, x_sem.at[1])
            wait(phase[2])

        prog = _interleave([(j, c) for c in range(HEAD_COLS) for j in range(j1)], [], 0)
        prog = _join(prog, sync2, _interleave(
            [(j, c) for c in range(HEAD_COLS, nc) for j in range(j1)]
            + pieces[j1 * nc:j2 * nc], [], 0))
        prog = _join(prog, sync3, _interleave(pieces[j2 * nc:], pieces, 0))
        run(0, x_even, prog, None)

        def tile(i, x_buf):
            seq_start = i % tiles_per_seq == 0
            seq_end = i % tiles_per_seq == tiles_per_seq - 1
            for c in range(nc):
                h_v[c, 0:HALO, :] = jnp.where(seq_start, 0.0, h_v[c, TILE:TILE + HALO, :])
                h_v[c, HALO:HALO + AHEAD, :] = carry_v[c]
            run(i, x_buf, _interleave(pieces, pieces, C_LAG), seq_end)

        def two_tiles(p, carry):
            more = p < tiles // 2 - 1

            @pl.when(more)
            def _():
                start_x_tile(2 * p + 2, x_even, x_sem.at[0])

            wait_x_tile(x_odd, x_sem.at[1])
            tile(2 * p + 1, x_odd)

            @pl.when(more)
            def _():
                start_x_tile(2 * p + 3, x_odd, x_sem.at[1], may_be_last=True)
                wait_x_tile(x_even, x_sem.at[0])
                tile(2 * p + 2, x_even)

            return carry

        lax.fori_loop(0, tiles // 2, two_tiles, None)
        pltpu.make_async_copy(o_v, o_v, o_sem).wait()

    out = pl.pallas_call(
        kernel,
        in_specs=[pl.BlockSpec(memory_space=pl.ANY)] * 4,
        out_specs=pl.BlockSpec(memory_space=pl.ANY),
        out_shape=jax.ShapeDtypeStruct((rows, dim), bf16),
        scratch_shapes=[
            pltpu.VMEM((nc, AHEAD + TILE, LANES), bf16),
            pltpu.VMEM((nc, AHEAD + TILE, LANES), bf16),
            pltpu.VMEM((2 * nc, dim, LANES), bf16),
            pltpu.VMEM((taps, dim), bf16),
            pltpu.VMEM((nc, dim, LANES), bf16),
            pltpu.VMEM((taps, dim), f32),
            pltpu.VMEM((nc, rows, LANES), bf16),
            pltpu.VMEM((nc, TILE + 2 * HALO, LANES), f32),
            pltpu.VMEM((nc, AHEAD, LANES), f32),
            pltpu.SemaphoreType.DMA((4,)),
            pltpu.SemaphoreType.DMA((2,)),
            pltpu.SemaphoreType.DMA(()),
        ],
        compiler_params=pltpu.CompilerParams(
            vmem_limit_bytes=64 * 1024 * 1024,
            disable_bounds_checks=True,
        ),
    )(x.reshape(rows, dim), w_pw1, dw, w_pw2)
    return out.reshape(batch, seq, dim)
```

```python
import jax
import jax.numpy as jnp
from jax import lax
import jax.experimental.pallas as pl
import jax.experimental.pallas.tpu as pltpu

LANES = 128
CHUNK = 80
CHUNKS = 25
TILE = CHUNK * CHUNKS
AHEAD = 16
HALO = 8
UNIT = 16
C_LAG = 12
X_GROUPS = (0, 9, 15, 20, 24, 25)
OUT_GROUPS = (0, 6, 12, 17, 20, 23, 24, 25)
OUT_LATE = 17
HEAD_COLS = 2
HEAD_GROUPS = (0, 3, 4, 9, 25)


def _interleave(a_pieces, c_pieces=(), lag=0):
    prog = []
    todo = list(c_pieces)
    for n, (j, c) in enumerate(a_pieces):
        prog += [("A", j, c), ("B", j, c)]
        if n >= lag and todo:
            prog.append(("C",) + todo.pop(0))
    return prog + [("C",) + p for p in todo]


def _join(prog, sync, rest):
    if prog[-1][0] == "B":
        return prog[:-1] + [sync, prog[-1]] + rest
    return prog + [sync] + rest


@jax.jit
def pallas_standalone__conformer_conv_module__speech_kernel(
    x: jax.Array,
    w_pw1: jax.Array,
    dw: jax.Array,
    w_pw2: jax.Array,
):
    batch, seq, dim = x.shape
    taps = dw.shape[0]
    pad = taps // 2
    rows = batch * seq
    nc = dim // LANES
    tiles = rows // TILE
    tiles_per_seq = seq // TILE
    assert dim == 4 * LANES and 1 <= pad <= HALO
    assert seq % TILE == 0 and tiles_per_seq > 1
    f32, bf16, u32 = jnp.float32, jnp.bfloat16, jnp.uint32
    pieces = [(j, c) for j in range(CHUNKS) for c in range(nc)]
    phases = len(HEAD_GROUPS) - 1

    def kernel(x_hbm, w1_hbm, dw_hbm, w2_hbm, o_hbm,
               w1_v, dw_v, w2_v, dw_f, o_v, h_v, carry_v, s_v, x_v,
               head_sem, x_sem, o_sem):
        def cols(c):
            return pl.ds(c * LANES, LANES)

        def aligned(r):
            return r if isinstance(r, int) else pl.multiple_of(r, AHEAD)

        def start(copies):
            for cp in copies:
                cp.start()

        def wait(copies):
            for cp in copies:
                cp.wait()

        def x_copies(src_row, dst_row, n, sem):
            return [
                pltpu.make_async_copy(
                    x_hbm.at[pl.ds(aligned(src_row), n), cols(c)],
                    x_v.at[c, pl.ds(dst_row, n)], sem)
                for c in range(nc)
            ]

        def refill(i, j0, j1):
            lo, hi = AHEAD + j0 * CHUNK, AHEAD + j1 * CHUNK
            if j1 < CHUNKS or isinstance(i, int):
                start(x_copies(i * TILE + lo, lo, hi - lo, x_sem))
                return
            start(x_copies(i * TILE + lo, lo, TILE - lo, x_sem))
            start(x_copies(jnp.minimum((i + 1) * TILE, rows - AHEAD), TILE, AHEAD, x_sem))

        def write_back(i, j0, j1, c):
            span = pl.ds(aligned(i * TILE + j0 * CHUNK), (j1 - j0) * CHUNK)
            pltpu.make_async_copy(o_v.at[c, span], o_hbm.at[span, cols(c)], o_sem).start()

        def packed(v):
            return pltpu.bitcast(v, bf16)

        x_w, s_w = x_v.bitcast(u32), s_v.bitcast(u32)
        w1_w, w2_w = w1_v.bitcast(u32), w2_v.bitcast(u32)

        def load_never():
            zeros = x_w[0, pl.ds((AHEAD + TILE) // 2, 8), :]
            return jnp.concatenate([zeros] * (UNIT // 8), axis=0) != 0

        def run(i, prog, seq_end):
            head = isinstance(i, int)
            a_done = [0] * CHUNKS
            never = load_never()
            last_h = last_y = None

            def piece_a(j, c):
                nonlocal last_h, never
                lo = 0 if head and j == 0 else AHEAD + j * CHUNK
                hi = AHEAD + (j + 1) * CHUNK
                xt = jnp.concatenate(
                    [packed(x_w[k, lo // 2:hi // 2, :]) for k in range(nc)], axis=1)
                b = jnp.dot(xt, packed(w1_w[nc + c]), preferred_element_type=f32)
                a = jnp.dot(xt, packed(w1_w[c]), preferred_element_type=f32)
                h = a * jnp.tanh(b * 0.5) + a
                last_h = h[hi - lo - UNIT:]
                if j < CHUNKS - 1:
                    h_v[c, HALO + lo:HALO + hi, :] = h
                else:
                    own = CHUNK - AHEAD
                    nxt = h[own:own + HALO]
                    h_v[c, HALO + lo:HALO + TILE, :] = h[:own]
                    h_v[c, HALO + TILE:, :] = nxt if head else jnp.where(seq_end, 0.0, nxt)
                    carry_v[c] = h[own:]

                a_done[j] += 1
                j0 = max(g for g in X_GROUPS if g <= j)
                j1 = min(g for g in X_GROUPS if g > j)
                if all(n == nc for n in a_done[j0:j1]):
                    if head:
                        refill(1, j0, j1)
                    else:
                        pl.when(i < tiles - 1)(lambda: refill(i + 1, j0, j1))
                    if j1 == CHUNKS:
                        never = load_never()

            def piece_b(j, c):
                nonlocal last_h, last_y
                w = [dw_f[k:k + 1, cols(c)] for k in range(taps)]
                parts = []
                for r in range(j * CHUNK, (j + 1) * CHUNK, UNIT):
                    y = None
                    for k in range(taps):
                        t = h_v[c, pl.ds(HALO - pad + r + k, UNIT), :] * w[k]
                        if k == 0 and last_y is not None:
                            t = jnp.where(never, last_y, t)
                        if k == 1 and last_h is not None:
                            t = jnp.where(never, last_h, t)
                            last_h = None
                        y = t if y is None else y + t
                    last_y = y
                    parts.append(y * jnp.tanh(y) + y)
                s_v[c, j * CHUNK:(j + 1) * CHUNK, :] = (
                    jnp.concatenate(parts, axis=0).astype(bf16))

            def piece_c(j, c):
                lo, hi = j * CHUNK, (j + 1) * CHUNK
                st = jnp.concatenate(
                    [packed(s_w[k, lo // 2:hi // 2, :]) for k in range(nc)], axis=1)
                out = jnp.dot(st, packed(w2_w[c]), preferred_element_type=f32)
                o_v[c, pl.ds(aligned(i * TILE + lo), CHUNK), :] = out.astype(bf16)
                if j + 1 in OUT_GROUPS:
                    j0 = OUT_GROUPS[OUT_GROUPS.index(j + 1) - 1]
                    if j0 < OUT_LATE:
                        write_back(i, j0, j + 1, c)
                    elif not head:
                        pl.when(i == tiles - 1)(lambda: write_back(i, j0, j + 1, c))

            for op in prog:
                if callable(op):
                    op()
                    last_h = last_y = None
                else:
                    {"A": piece_a, "B": piece_b, "C": piece_c}[op[0]](op[1], op[2])

        def head_copies(p):
            sem = head_sem.at[p]
            lo = AHEAD + HEAD_GROUPS[p] * CHUNK if p else 0
            hi = AHEAD + HEAD_GROUPS[p + 1] * CHUNK
            blocks = [range(HEAD_COLS), range(HEAD_COLS, nc)]
            copies = x_copies(lo, lo, hi - lo, sem)
            if p < 2:
                copies += [
                    pltpu.make_async_copy(w1_hbm.at[:, cols(q)], w1_v.at[q], sem)
                    for c in blocks[p] for q in (nc + c, c)
                ]
            if p == 2:
                copies += [
                    pltpu.make_async_copy(w2_hbm.at[:, cols(c)], w2_v.at[c], sem)
                    for c in range(nc)
                ]
            return copies

        def head_sync(p):
            def sync():
                if 2 <= p < phases - 1:
                    start(head_copies(p + 1))
                wait(head_copies(p))
            return sync

        x_v[0, AHEAD + TILE:, :] = jnp.zeros((AHEAD, LANES), bf16)
        dw_copy = pltpu.make_async_copy(dw_hbm, dw_v, x_sem)
        dw_copy.start()
        for p in range(3):
            start(head_copies(p))
        for c in range(nc):
            h_v[c, 0:HALO, :] = jnp.zeros((HALO, LANES), f32)
        dw_copy.wait()
        dw_f[...] = dw_v[...].astype(f32) * 0.25
        wait(head_copies(0))

        j1, j2 = HEAD_GROUPS[1:3]
        prog = _interleave([(j, c) for c in range(HEAD_COLS) for j in range(j1)])
        prog = _join(prog, head_sync(1), _interleave(
            [(j, c) for c in range(HEAD_COLS, nc) for j in range(j1)]
            + pieces[j1 * nc:j2 * nc]))
        c_done = 0
        for p in range(2, phases):
            lo, hi = HEAD_GROUPS[p] * nc, HEAD_GROUPS[p + 1] * nc
            c_end = hi if p == phases - 1 else hi - C_LAG
            prog = _join(prog, head_sync(p),
                         _interleave(pieces[lo:hi], pieces[c_done:c_end]))
            c_done = c_end
        run(0, prog, None)

        def tile(i, carry):
            filled = x_v.at[:, pl.ds(AHEAD, TILE)]
            pltpu.make_async_copy(filled, filled, x_sem).wait()
            for c in range(nc):
                write_back(i - 1, OUT_LATE, CHUNKS, c)
            pos = lax.rem(i, tiles_per_seq)
            for c in range(nc):
                h_v[c, 0:HALO, :] = jnp.where(pos == 0, 0.0, h_v[c, TILE:TILE + HALO, :])
                h_v[c, HALO:HALO + AHEAD, :] = carry_v[c]
            run(i, _interleave(pieces, pieces, C_LAG), pos == tiles_per_seq - 1)
            return carry

        lax.fori_loop(1, tiles, tile, None)
        pltpu.make_async_copy(o_hbm, o_hbm, o_sem).wait()

    out = pl.pallas_call(
        kernel,
        in_specs=[pl.BlockSpec(memory_space=pl.ANY)] * 4,
        out_specs=pl.BlockSpec(memory_space=pl.ANY),
        out_shape=jax.ShapeDtypeStruct((rows, dim), bf16),
        scratch_shapes=[
            pltpu.VMEM((2 * nc, dim, LANES), bf16),
            pltpu.VMEM((taps, dim), bf16),
            pltpu.VMEM((nc, dim, LANES), bf16),
            pltpu.VMEM((taps, dim), f32),
            pltpu.VMEM((nc, rows, LANES), bf16),
            pltpu.VMEM((nc, TILE + 2 * HALO, LANES), f32),
            pltpu.VMEM((nc, AHEAD, LANES), f32),
            pltpu.VMEM((nc, TILE, LANES), bf16),
            pltpu.VMEM((nc, TILE + 2 * AHEAD, LANES), bf16),
            pltpu.SemaphoreType.DMA((phases,)),
            pltpu.SemaphoreType.DMA(()),
            pltpu.SemaphoreType.DMA(()),
        ],
        compiler_params=pltpu.CompilerParams(
            vmem_limit_bytes=64 * 1024 * 1024,
            disable_bounds_checks=True,
        ),
    )(x.reshape(rows, dim), w_pw1, dw, w_pw2)
    return out.reshape(batch, seq, dim)
```

```python
import jax
import jax.numpy as jnp
from jax import lax
import jax.experimental.pallas as pl
import jax.experimental.pallas.tpu as pltpu

LANES = 128
CHUNK = 80
CHUNKS = 25
TILE = CHUNK * CHUNKS
AHEAD = 16
HALO = 8
UNIT = 16
C_LAG = 12
X_GROUPS = (0, 9, 15, 20, 24, 25)
OUT_GROUPS = (0, 6, 12, 17, 20, 23, 24, 25)
OUT_LATE = 17
HEAD_COLS = 2
HEAD_GROUPS = (0, 3, 4, 9, 25)


def _interleave(a_pieces, c_pieces=(), lag=0):
    prog = []
    todo = list(c_pieces)
    for n, (j, c) in enumerate(a_pieces):
        prog += [("A", j, c), ("B", j, c)]
        if n >= lag and todo:
            prog.append(("C",) + todo.pop(0))
    return prog + [("C",) + p for p in todo]


def _join(prog, sync, rest):
    if prog[-1][0] == "B":
        return prog[:-1] + [sync, prog[-1]] + rest
    return prog + [sync] + rest


@jax.jit
def pallas_standalone__conformer_conv_module__speech_kernel(
    x: jax.Array,
    w_pw1: jax.Array,
    dw: jax.Array,
    w_pw2: jax.Array,
):
    batch, seq, dim = x.shape
    taps = dw.shape[0]
    pad = taps // 2
    rows = batch * seq
    nc = dim // LANES
    tiles = rows // TILE
    tiles_per_seq = seq // TILE
    assert dim == 4 * LANES and 1 <= pad <= HALO
    assert seq % TILE == 0 and tiles_per_seq > 1 and tiles > 2
    f32, bf16, u32 = jnp.float32, jnp.bfloat16, jnp.uint32
    pieces = [(j, c) for j in range(CHUNKS) for c in range(nc)]
    phases = len(HEAD_GROUPS) - 1

    def kernel(x_hbm, w1_hbm, dw_hbm, w2_hbm, o_hbm,
               x_v, w1_v, dw_v, w2_v, w_pk, dw_f, h_v, carry_v, s_v, o_v,
               in_sem, o_sem):
        x_sem = in_sem.at[phases]

        def cols(c):
            return pl.ds(c * LANES, LANES)

        def aligned(r):
            return r if isinstance(r, int) else pl.multiple_of(r, AHEAD)

        def start(copies):
            for cp in copies:
                cp.start()

        def wait(copies):
            for cp in copies:
                cp.wait()

        def x_copy(src_row, dst_row, n, sem):
            return pltpu.make_async_copy(
                x_hbm.at[pl.ds(aligned(src_row), n)], x_v.at[pl.ds(dst_row, n)], sem)

        def refill(i, j0, j1):
            lo, hi = AHEAD + j0 * CHUNK, AHEAD + j1 * CHUNK
            if j1 < CHUNKS or isinstance(i, int):
                x_copy(i * TILE + lo, lo, hi - lo, x_sem).start()
                return
            x_copy(i * TILE + lo, lo, TILE - lo, x_sem).start()
            x_copy(jnp.minimum((i + 1) * TILE, rows - AHEAD), TILE, AHEAD, x_sem).start()

        def write_back(i, j0, j1, c):
            span = pl.ds(aligned(i * TILE + j0 * CHUNK), (j1 - j0) * CHUNK)
            pltpu.make_async_copy(o_v.at[c, span], o_hbm.at[span, cols(c)], o_sem).start()

        repacked = []

        def weight(q):
            if q in repacked:
                return pltpu.bitcast(w_pk[q], bf16)
            w = w1_v[q] if q < 2 * nc else w2_v[:, cols(q - 2 * nc)]
            w_pk[q] = pltpu.bitcast(w, u32)
            repacked.append(q)
            return w

        def load_never():
            return x_v[AHEAD + TILE:, cols(0)].astype(f32) != 0.0

        def run(i, prog, seq_end):
            head = isinstance(i, int)
            a_done = [0] * CHUNKS
            never = load_never()
            last_h = last_y = None

            def piece_a(j, c):
                nonlocal last_h, never
                lo = 0 if head and j == 0 else AHEAD + j * CHUNK
                hi = AHEAD + (j + 1) * CHUNK
                xt = x_v[lo:hi, :]
                b = jnp.dot(xt, weight(nc + c), preferred_element_type=f32)
                a = jnp.dot(xt, weight(c), preferred_element_type=f32)
                h = a * jnp.tanh(b * 0.5) + a
                last_h = h[hi - lo - UNIT:]
                if j < CHUNKS - 1:
                    h_v[c, HALO + lo:HALO + hi, :] = h
                else:
                    own = CHUNK - AHEAD
                    nxt = h[own:own + HALO]
                    h_v[c, HALO + lo:HALO + TILE, :] = h[:own]
                    h_v[c, HALO + TILE:, :] = nxt if head else jnp.where(seq_end, 0.0, nxt)
                    carry_v[c] = h[own:]

                a_done[j] += 1
                j0 = max(g for g in X_GROUPS if g <= j)
                j1 = min(g for g in X_GROUPS if g > j)
                if all(n == nc for n in a_done[j0:j1]):
                    if head:
                        refill(1, j0, j1)
                    else:
                        pl.when(i < tiles - 1)(lambda: refill(i + 1, j0, j1))
                    if j1 == CHUNKS:
                        never = load_never()

            def piece_b(j, c):
                nonlocal last_h, last_y
                w = [dw_f[k:k + 1, cols(c)] for k in range(taps)]
                parts = []
                for r in range(j * CHUNK, (j + 1) * CHUNK, UNIT):
                    y = None
                    for k in range(taps):
                        t = h_v[c, pl.ds(HALO - pad + r + k, UNIT), :] * w[k]
                        if k == 0 and last_y is not None:
                            t = jnp.where(never, last_y, t)
                        if k == 1 and last_h is not None:
                            t = jnp.where(never, last_h, t)
                            last_h = None
                        y = t if y is None else y + t
                    last_y = y
                    parts.append(y * jnp.tanh(y) + y)
                s_v[c, j * CHUNK:(j + 1) * CHUNK, :] = (
                    jnp.concatenate(parts, axis=0).astype(bf16))

            def piece_c(j, c):
                lo, hi = j * CHUNK, (j + 1) * CHUNK
                st = jnp.concatenate([s_v[k, lo:hi, :] for k in range(nc)], axis=1)
                out = jnp.dot(st, weight(2 * nc + c), preferred_element_type=f32)
                o_v[c, pl.ds(aligned(i * TILE + lo), CHUNK), :] = out.astype(bf16)
                if j + 1 in OUT_GROUPS:
                    j0 = OUT_GROUPS[OUT_GROUPS.index(j + 1) - 1]
                    if j0 < OUT_LATE:
                        write_back(i, j0, j + 1, c)
                    elif not head:
                        pl.when(i == tiles - 1)(lambda: write_back(i, j0, j + 1, c))

            for op in prog:
                if callable(op):
                    op()
                    last_h = last_y = None
                else:
                    {"A": piece_a, "B": piece_b, "C": piece_c}[op[0]](op[1], op[2])

        def head_copies(p):
            sem = in_sem.at[p]
            lo = AHEAD + HEAD_GROUPS[p] * CHUNK if p else 0
            hi = AHEAD + HEAD_GROUPS[p + 1] * CHUNK
            copies = [x_copy(lo, lo, hi - lo, sem)]
            if p < 2:
                blocks = range(HEAD_COLS, nc) if p else range(HEAD_COLS)
                copies += [
                    pltpu.make_async_copy(w1_hbm.at[:, cols(q)], w1_v.at[q], sem)
                    for c in blocks for q in (nc + c, c)
                ]
            if p == 2:
                copies.append(pltpu.make_async_copy(w2_hbm, w2_v, sem))
            return copies

        def head_sync(p):
            def sync():
                if 2 <= p < phases - 1:
                    start(head_copies(p + 1))
                wait(head_copies(p))
            return sync

        x_v[AHEAD + TILE:, cols(0)] = jnp.zeros((UNIT, LANES), bf16)
        dw_copy = pltpu.make_async_copy(dw_hbm, dw_v, x_sem)
        dw_copy.start()
        for p in range(3):
            start(head_copies(p))
        for c in range(nc):
            h_v[c, 0:HALO, :] = jnp.zeros((HALO, LANES), f32)
        dw_copy.wait()
        dw_f[...] = dw_v[...].astype(f32) * 0.25
        wait(head_copies(0))

        j1, j2 = HEAD_GROUPS[1:3]
        prog = _interleave([(j, c) for c in range(HEAD_COLS) for j in range(j1)])
        prog = _join(prog, head_sync(1), _interleave(
            [(j, c) for c in range(HEAD_COLS, nc) for j in range(j1)]
            + pieces[j1 * nc:j2 * nc]))
        c_done = 0
        for p in range(2, phases):
            lo, hi = HEAD_GROUPS[p] * nc, HEAD_GROUPS[p + 1] * nc
            c_end = hi if p == phases - 1 else hi - C_LAG
            prog = _join(prog, head_sync(p),
                         _interleave(pieces[lo:hi], pieces[c_done:c_end]))
            c_done = c_end
        run(0, prog, None)

        def tile(i, carry):
            filled = x_v.at[pl.ds(AHEAD, TILE)]
            pltpu.make_async_copy(filled, filled, x_sem).wait()
            for c in range(nc):
                write_back(i - 1, OUT_LATE, CHUNKS, c)
            pos = lax.rem(i, tiles_per_seq)
            for c in range(nc):
                h_v[c, 0:HALO, :] = jnp.where(pos == 0, 0.0, h_v[c, TILE:TILE + HALO, :])
                h_v[c, HALO:HALO + AHEAD, :] = carry_v[c]
            run(i, _interleave(pieces, pieces, C_LAG), pos == tiles_per_seq - 1)
            return carry

        lax.fori_loop(1, tiles, tile, None)
        pltpu.make_async_copy(o_hbm, o_hbm, o_sem).wait()

    out = pl.pallas_call(
        kernel,
        in_specs=[pl.BlockSpec(memory_space=pl.ANY)] * 4,
        out_specs=pl.BlockSpec(memory_space=pl.ANY),
        out_shape=jax.ShapeDtypeStruct((rows, dim), bf16),
        scratch_shapes=[
            pltpu.VMEM((AHEAD + TILE + UNIT, dim), bf16),
            pltpu.VMEM((2 * nc, dim, LANES), bf16),
            pltpu.VMEM((taps, dim), bf16),
            pltpu.VMEM((dim, dim), bf16),
            pltpu.VMEM((3 * nc, dim // 2, LANES), u32),
            pltpu.VMEM((taps, dim), f32),
            pltpu.VMEM((nc, TILE + 2 * HALO, LANES), f32),
            pltpu.VMEM((nc, AHEAD, LANES), f32),
            pltpu.VMEM((nc, TILE, LANES), bf16),
            pltpu.VMEM((nc, rows, LANES), bf16),
            pltpu.SemaphoreType.DMA((phases + 1,)),
            pltpu.SemaphoreType.DMA(()),
        ],
        compiler_params=pltpu.CompilerParams(
            vmem_limit_bytes=64 * 1024 * 1024,
            disable_bounds_checks=True,
        ),
    )(x.reshape(rows, dim), w_pw1, dw, w_pw2)
    return out.reshape(batch, seq, dim)
```
